```python
import jax
import jax.numpy as jnp

def _softmax(x, axis=-1):
    return jax.nn.softmax(x, axis=axis)

def _gelu(x):
    return jax.nn.gelu(x, approximate=True)

def _silu(x):
    return jax.nn.silu(x)

def _sigmoid(x):
    return jax.nn.sigmoid(x)

def _layernorm(x, axis=-1, eps=1e-05):
    m = jnp.mean(x, axis=axis, keepdims=True)
    v = jnp.var(x, axis=axis, keepdims=True)
    return (x - m) / jnp.sqrt(v + eps)

def _scatter_add(tgt, idx, src, axis=0):
    return tgt.at[idx].add(src)

def _segment_sum(src, seg, n):
    return jax.ops.segment_sum(src, seg, n)

class _Rng:

    def __init__(self, key):
        self._k = key

    def _next(self):
        self._k, sub = jax.random.split(self._k)
        return sub

    def normal(self, shape):
        return jax.random.normal(self._next(), shape, dtype=jnp.bfloat16)

    def randint(self, lo, hi, shape):
        return jax.random.randint(self._next(), shape, lo, hi, dtype=jnp.int32)

    def uniform(self, shape, lo=0.0, hi=1.0):
        return jax.random.uniform(self._next(), shape, jnp.bfloat16, lo, hi)

    def permutation(self, n):
        return jax.random.permutation(self._next(), n)
kernel_name = 'adaLN_cond__ssm_conv_h3__dense_activation_gelu__prompt'

def setup_inputs():
    _rng = _Rng(jax.random.key(int.from_bytes(__import__("os").urandom(4), "little")))
    _w = lambda a: (lambda t: t.astype(jnp.bfloat16) if jnp.issubdtype(t.dtype, jnp.floating) else t)(jnp.asarray(a))

    def _A_setup():
        B, S, D = (1, 2048, 640)
        ks = 4
        return {'q': _w((lambda *s: _rng.normal(s) * 0.05)(B, S, D)), 'k': _w((lambda *s: _rng.normal(s) * 0.05)(B, S, D)), 'v': _w((lambda *s: _rng.normal(s) * 0.05)(B, S, D)), 'shift_k': _w((lambda *s: _rng.normal(s) * 0.05)(D, ks) * 0.5), 'ssm_k': _w((lambda *s: _rng.normal(s) * 0.05)(D, S) * (1.0 / S ** 0.5)), 'ssm_D': _w((lambda *s: _rng.normal(s) * 0.05)(D))}
    _A_in = _A_setup()

    def _B_setup():
        B, S, D, F = (1, 2048, 640, 1728)
        return {'x': _w((lambda *s: _rng.normal(s) * 0.05)(B, S, D)), 'w1': _w((lambda *s: _rng.normal(s) * 0.05)(D, F) * D ** (-0.5)), 'b1': _w((lambda *s: _rng.normal(s) * 0.05)(F) * 0.01), 'w2': _w((lambda *s: _rng.normal(s) * 0.05)(F, D) * F ** (-0.5)), 'b2': _w((lambda *s: _rng.normal(s) * 0.05)(D) * 0.01)}
    _B_in = _B_setup()
    return {'A_q': _A_in['q'], 'A_k': _A_in['k'], 'A_v': _A_in['v'], 'A_shift_k': _A_in['shift_k'], 'A_ssm_k': _A_in['ssm_k'], 'A_ssm_D': _A_in['ssm_D'], 'B_x': _B_in['x'], 'B_w1': _B_in['w1'], 'B_b1': _B_in['b1'], 'B_w2': _B_in['w2'], 'B_b2': _B_in['b2'], 'c': _w((lambda *s: _rng.normal(s) * 0.05)(1, 640)), 'w_mod': _w((lambda *s: _rng.normal(s) * 0.05)(640, 6 * 640) * 640 ** (-0.5))}

def reference(A_q, A_k, A_v, A_shift_k, A_ssm_k, A_ssm_D, B_x, B_w1, B_b1, B_w2, B_b2, c, w_mod):

    def _A_ref(q, k, v, shift_k, ssm_k, ssm_D):
        B, S, D = q.shape
        ks = shift_k.shape[-1]
        k_pad = jnp.pad(k, ((0, 0), (ks - 1, 0), (0, 0)))
        k_shift = jnp.zeros_like(k)
        for t in range(ks):
            k_shift = k_shift + k_pad[:, t:t + S, :] * shift_k[:, ks - 1 - t][None, None, :]
        kv = k_shift * v
        L = 2 * S
        kv_pad = jnp.pad(kv, ((0, 0), (0, S), (0, 0)))
        kf_pad = jnp.pad(ssm_k, ((0, 0), (0, S)))
        kv_f = (lambda x, axes=(-2, -1): jnp.fft.rfft2(x.astype(jnp.float32), axes=axes))(kv_pad[:, None, :, :], axes=(1, 2))
        kf_f = (lambda x, axes=(-2, -1): jnp.fft.rfft2(x.astype(jnp.float32), axes=axes))(kf_pad[:, None, :], axes=(1, 2))
        kf_f = (lambda x, *d: x.transpose(*d))(kf_f, 1, 2, 0)
        y_f = kv_f * kf_f[None, :, :, :]
        y = (lambda x, s, axes=(-2, -1): jnp.fft.irfft2(x, s=s, axes=axes).astype(jnp.bfloat16))(y_f, (1, L), axes=(1, 2))[:, 0, :S, :]
        y = y + kv * ssm_D[None, None, :]
        return q * y

    def _B_ref(x, w1, b1, w2, b2):
        h = jnp.einsum('bsd,df->bsf', x, w1) + b1
        h = _gelu(h)
        return jnp.einsum('bsf,fd->bsd', h, w2) + b2
    x = A_q
    mod = (_silu(c) @ w_mod).reshape(c.shape[0], 6, 1, -1)
    sa, ca, ga, sb, cb, gb = (mod[:, 0].copy(), mod[:, 1].copy(), mod[:, 2].copy(), mod[:, 3].copy(), mod[:, 4].copy(), mod[:, 5].copy())
    h = _layernorm(x, axis=-1) * (1 + ca) + sa
    x = x + ga * _A_ref(h, A_k, A_v, A_shift_k, A_ssm_k, A_ssm_D)
    h = _layernorm(x, axis=-1) * (1 + cb) + sb
    x = x + gb * _B_ref(h, B_w1, B_b1, B_w2, B_b2)
    return x
```

```python
import functools

import jax
import jax.numpy as jnp
import numpy as np
import jax.experimental.pallas as pl
import jax.experimental.pallas.tpu as pltpu

_T = 128
_LANES = 128
_ROWS = 256
_EPS = 1e-5


def _dft_matrices():
    k = np.concatenate([np.arange(0, _T, 2), np.arange(1, _T, 2)])
    t = np.arange(_T)
    phase = ((2 * k[:, None] + 1) * t[None, :]) % (4 * _T)
    ang = phase.astype(np.float64) * (2.0 * np.pi / (4 * _T))
    fwd = np.concatenate([np.cos(ang), -np.sin(ang)], axis=0)
    inv = fwd.T / _T
    return fwd.astype(np.float32), inv.astype(np.float32)


_FWD_NP, _INV_NP = _dft_matrices()


def _layernorm(x):
    m = jnp.mean(x, axis=-1, keepdims=True)
    d = x - m
    v = jnp.mean(d * d, axis=-1, keepdims=True)
    return d * jax.lax.rsqrt(v + _EPS)


def _gelu(x):
    c0 = float(np.sqrt(2.0 / np.pi))
    inner = x * (c0 + (c0 * 0.044715) * (x * x))
    hx = 0.5 * x
    return hx + hx * jnp.tanh(inner)


def _toeplitz(u, k):
    out = []
    for i in range(len(u)):
        acc = u[0] * k[i]
        for j in range(1, i + 1):
            acc = acc + u[j] * k[i - j]
        out.append(acc)
    return out


def _kernel(q_hbm, k_hbm, v_hbm, shift_ref, ssmk_hbm, ssmd_ref, w1_hbm, b1_ref,
            w2_hbm, b2_ref, c_ref, wmod_hbm, fwd_hbm, inv_hbm, out_hbm,
            kbuf, vbuf, sbuf, qbuf, obuf, w1buf, w2buf, wmbuf, fwd, inv,
            taps, kvbuf, uspec, kspec, yspec, ybuf, modbuf,
            sem_k, sem_v, sem_s, sem_w, sem_o):
    S, D = qbuf.shape
    nslab = D // _LANES
    nblk = S // _T
    f32, bf16 = jnp.float32, jnp.bfloat16

    def slab_copies(c):
        lo = pl.multiple_of(c * _LANES, _LANES)
        return (
            pltpu.make_async_copy(k_hbm.at[:, pl.ds(lo, _LANES)], kbuf.at[c], sem_k.at[c]),
            pltpu.make_async_copy(v_hbm.at[:, pl.ds(lo, _LANES)], vbuf.at[c], sem_v.at[c]),
            pltpu.make_async_copy(ssmk_hbm.at[pl.ds(lo, _LANES), :], sbuf.at[c], sem_s.at[c]),
        )

    cp_fwd = pltpu.make_async_copy(fwd_hbm, fwd, sem_w.at[0])
    cp_inv = pltpu.make_async_copy(inv_hbm, inv, sem_w.at[1])
    cp_wm = pltpu.make_async_copy(wmod_hbm, wmbuf, sem_w.at[2])
    cp_w1 = pltpu.make_async_copy(w1_hbm, w1buf, sem_w.at[3])
    cp_w2 = pltpu.make_async_copy(w2_hbm, w2buf, sem_w.at[4])
    cp_q = pltpu.make_async_copy(q_hbm, qbuf, sem_w.at[5])

    cp_fwd.start()
    for cp in slab_copies(0):
        cp.start()
    cp_inv.start()
    for c in range(1, nslab):
        for cp in slab_copies(c):
            cp.start()
    cp_wm.start()
    cp_q.start()
    cp_w1.start()
    cp_w2.start()

    sh_t = jnp.transpose(shift_ref[...].astype(f32))
    dvec = ssmd_ref[...].astype(f32)
    for c in range(nslab):
        sl = slice(c * _LANES, (c + 1) * _LANES)
        for j in range(4):
            taps[c, j] = jnp.broadcast_to(sh_t[j:j + 1, sl], (8, _LANES))
        taps[c, 4] = jnp.broadcast_to(dvec[:, sl], (8, _LANES))

    cp_fwd.wait()
    cp_inv.wait()

    def slab_body(c, carry):
        for cp in slab_copies(c):
            cp.wait()
        fmat = fwd[...]
        tap = [taps[c, j][0:1, :] for j in range(4)]
        prev = jnp.zeros((8, _LANES), f32)
        for j in range(nblk):
            rows = slice(j * _T, (j + 1) * _T)
            kc = kbuf[c, rows, :].astype(f32)
            ext = jnp.concatenate([prev, kc], axis=0)
            ks = kc * tap[0]
            for s in range(1, 4):
                ks = ks + ext[8 - s:8 - s + _T, :] * tap[s]
            prev = kc[_T - 8:, :]
            kv = ks * vbuf[c, rows, :].astype(f32)
            kvbuf[rows, :] = kv
            uspec[j] = jnp.dot(fmat, kv.astype(bf16), preferred_element_type=f32)
            kspec[j] = jax.lax.dot_general(
                fmat, sbuf[c, :, rows], (((1,), (1,)), ((), ())),
                preferred_element_type=f32)

        def make_pos_body(sign):
            def pos_body(p, carry2):
                re = pl.ds(pl.multiple_of(p * 8, 8), 8)
                im = pl.ds(pl.multiple_of(p * 8 + _T, 8), 8)
                kre = [kspec[m, re, :] for m in range(nblk)]
                kim = [kspec[m, im, :] for m in range(nblk)]
                cc, dd = [kre[0]], [kim[0]]
                for m in range(1, nblk):
                    if sign > 0:
                        cc.append(kre[m] - kim[m - 1])
                        dd.append(kim[m] + kre[m - 1])
                    else:
                        cc.append(kre[m] + kim[m - 1])
                        dd.append(kim[m] - kre[m - 1])
                a = [uspec[j, re, :] for j in range(nblk)]
                b = [uspec[j, im, :] for j in range(nblk)]
                p1 = _toeplitz([x + y for x, y in zip(a, b)], cc)
                p2 = _toeplitz(a, [y - x for x, y in zip(cc, dd)])
                for i in range(nblk):
                    yspec[i, im, :] = p1[i] + p2[i]
                p3 = _toeplitz(b, [x + y for x, y in zip(cc, dd)])
                for i in range(nblk):
                    yspec[i, re, :] = p1[i] - p3[i]
                return carry2
            return pos_body

        half = _T // 16
        jax.lax.fori_loop(0, half, make_pos_body(1), 0)
        jax.lax.fori_loop(half, 2 * half, make_pos_body(-1), 0)

        gmat = inv[...]
        dskip = taps[c, 4][0:1, :]
        for i in range(nblk):
            rows = slice(i * _T, (i + 1) * _T)
            y = jnp.dot(gmat, yspec[i].astype(bf16), preferred_element_type=f32)
            ybuf[c, rows, :] = y + kvbuf[rows, :] * dskip
        return carry

    jax.lax.fori_loop(0, nslab, slab_body, 0)

    cp_wm.wait()
    cv = c_ref[...].astype(f32)
    sc = cv * (1.0 / (1.0 + jnp.exp(-cv)))
    sc8 = jnp.broadcast_to(sc, (8, D)).astype(bf16)
    modbuf[...] = jnp.dot(sc8, wmbuf[...], preferred_element_type=f32)

    cp_q.wait()
    cp_w1.wait()
    cp_w2.wait()

    def out_copy(r):
        rows = pl.ds(pl.multiple_of(r * _ROWS, _ROWS), _ROWS)
        return pltpu.make_async_copy(obuf.at[rows, :], out_hbm.at[rows, :], sem_o.at[r])

    def row_body(r, carry):
        rows = pl.ds(pl.multiple_of(r * _ROWS, _ROWS), _ROWS)
        mod = [modbuf[0:1, j * D:(j + 1) * D] for j in range(6)]
        sa, ca, ga, sb, cb, gb = mod
        x = qbuf[rows, :].astype(f32)
        y = jnp.concatenate([ybuf[c, rows, :] for c in range(nslab)], axis=1)
        h = _layernorm(x) * (1.0 + ca) + sa
        x2 = x + ga * (h * y)
        h2 = _layernorm(x2) * (1.0 + cb) + sb
        a = jnp.dot(h2.astype(bf16), w1buf[...], preferred_element_type=f32)
        a = _gelu(a + b1_ref[...].astype(f32))
        o = jnp.dot(a.astype(bf16), w2buf[...], preferred_element_type=f32)
        o = x2 + gb * (o + b2_ref[...].astype(f32))
        obuf[rows, :] = o.astype(obuf.dtype)
        out_copy(r).start()
        return carry

    nrow = S // _ROWS
    jax.lax.fori_loop(0, nrow, row_body, 0)
    for r in range(nrow):
        out_copy(r).wait()


@jax.jit
def pallas_adaLN_cond__ssm_conv_h3__dense_activation_gelu__prompt_kernel(
    A_q: jax.Array,
    A_k: jax.Array,
    A_v: jax.Array,
    A_shift_k: jax.Array,
    A_ssm_k: jax.Array,
    A_ssm_D: jax.Array,
    B_x: jax.Array,
    B_w1: jax.Array,
    B_b1: jax.Array,
    B_w2: jax.Array,
    B_b2: jax.Array,
    c: jax.Array,
    w_mod: jax.Array,
):
    del B_x
    B, S, D = A_q.shape
    F = B_w1.shape[1]
    assert B == 1 and S % _ROWS == 0 and D % _LANES == 0
    nslab, nblk = D // _LANES, S // _T
    f32, bf16 = jnp.float32, jnp.bfloat16

    hbm = pl.BlockSpec(memory_space=pl.ANY)
    vmem = pl.BlockSpec(memory_space=pltpu.VMEM)
    out = pl.pallas_call(
        _kernel,
        out_shape=jax.ShapeDtypeStruct((S, D), A_q.dtype),
        in_specs=[hbm, hbm, hbm, vmem, hbm, vmem, hbm, vmem, hbm, vmem, vmem, hbm, hbm, hbm],
        out_specs=hbm,
        scratch_shapes=[
            pltpu.VMEM((nslab, S, _LANES), bf16),
            pltpu.VMEM((nslab, S, _LANES), bf16),
            pltpu.VMEM((nslab, _LANES, S), bf16),
            pltpu.VMEM((S, D), bf16),
            pltpu.VMEM((S, D), A_q.dtype),
            pltpu.VMEM((D, F), bf16),
            pltpu.VMEM((F, D), bf16),
            pltpu.VMEM((D, 6 * D), bf16),
            pltpu.VMEM((2 * _T, _T), bf16),
            pltpu.VMEM((_T, 2 * _T), bf16),
            pltpu.VMEM((nslab, 5, 8, _LANES), f32),
            pltpu.VMEM((S, _LANES), f32),
            pltpu.VMEM((nblk, 2 * _T, _LANES), f32),
            pltpu.VMEM((nblk, 2 * _T, _LANES), f32),
            pltpu.VMEM((nblk, 2 * _T, _LANES), f32),
            pltpu.VMEM((nslab, S, _LANES), f32),
            pltpu.VMEM((8, 6 * D), f32),
            pltpu.SemaphoreType.DMA((nslab,)),
            pltpu.SemaphoreType.DMA((nslab,)),
            pltpu.SemaphoreType.DMA((nslab,)),
            pltpu.SemaphoreType.DMA((6,)),
            pltpu.SemaphoreType.DMA((S // _ROWS,)),
        ],
        compiler_params=pltpu.CompilerParams(vmem_limit_bytes=100 * 1024 * 1024),
    )(
        A_q.reshape(S, D), A_k.reshape(S, D), A_v.reshape(S, D), A_shift_k, A_ssm_k,
        A_ssm_D.reshape(1, D), B_w1, B_b1.reshape(1, F), B_w2, B_b2.reshape(1, D), c, w_mod,
        jnp.asarray(_FWD_NP, dtype=bf16), jnp.asarray(_INV_NP, dtype=bf16),
    )
    return out.reshape(B, S, D)
```

```python
import functools

import jax
import jax.numpy as jnp
import numpy as np
import jax.experimental.pallas as pl
import jax.experimental.pallas.tpu as pltpu

_T = 128
_LANES = 128
_ROWS = 256
_EPS = 1e-5


def _dft_matrices():
    k = np.concatenate([np.arange(0, _T, 2), np.arange(1, _T, 2)])
    t = np.arange(_T)
    phase = ((2 * k[:, None] + 1) * t[None, :]) % (4 * _T)
    ang = phase.astype(np.float64) * (2.0 * np.pi / (4 * _T))
    fwd = np.concatenate([np.cos(ang), -np.sin(ang)], axis=0)
    inv = fwd.T / _T
    return fwd.astype(np.float32), inv.astype(np.float32)


_FWD_NP, _INV_NP = _dft_matrices()


def _layernorm(x):
    m = jnp.mean(x, axis=-1, keepdims=True)
    d = x - m
    v = jnp.mean(d * d, axis=-1, keepdims=True)
    return d * jax.lax.rsqrt(v + _EPS)


def _gelu(x):
    c0 = float(np.sqrt(2.0 / np.pi))
    inner = x * (c0 + (c0 * 0.044715) * (x * x))
    hx = 0.5 * x
    return hx + hx * jnp.tanh(inner)


def _toeplitz(u, k):
    out = []
    for i in range(len(u)):
        acc = u[0] * k[i]
        for j in range(1, i + 1):
            acc = acc + u[j] * k[i - j]
        out.append(acc)
    return out


def _kernel(q_hbm, k_hbm, v_hbm, shift_hbm, ssmk_hbm, ssmd_hbm, w1t_hbm, b1_hbm,
            w2_hbm, b2_hbm, c_hbm, wmod_hbm, fwd_hbm, inv_hbm, out_hbm,
            shift_ref, ssmd_ref, b1_ref, b2_ref, c_ref,
            kbuf, vbuf, sbuf, qbuf, obuf, w1buf, w2buf, wmbuf, fwd, inv,
            taps, kvbuf, uspec, kspec, yspec, ybuf, modbuf,
            sem_k, sem_v, sem_s, sem_w, sem_o):
    S, D = qbuf.shape
    nslab = D // _LANES
    nblk = S // _T
    f32, bf16 = jnp.float32, jnp.bfloat16

    def slab_copies(c):
        lo = pl.multiple_of(c * _LANES, _LANES)
        return (
            pltpu.make_async_copy(k_hbm.at[:, pl.ds(lo, _LANES)], kbuf.at[c], sem_k.at[c]),
            pltpu.make_async_copy(v_hbm.at[:, pl.ds(lo, _LANES)], vbuf.at[c], sem_v.at[c]),
            pltpu.make_async_copy(ssmk_hbm.at[pl.ds(lo, _LANES), :], sbuf.at[c], sem_s.at[c]),
        )

    cp_fwd = pltpu.make_async_copy(fwd_hbm, fwd, sem_w.at[0])
    cp_inv = pltpu.make_async_copy(inv_hbm, inv, sem_w.at[1])
    cp_wm = pltpu.make_async_copy(wmod_hbm, wmbuf, sem_w.at[2])
    cp_w1 = pltpu.make_async_copy(w1t_hbm, w1buf, sem_w.at[3])
    cp_w2 = pltpu.make_async_copy(w2_hbm, w2buf, sem_w.at[4])
    cp_q = pltpu.make_async_copy(q_hbm, qbuf, sem_w.at[5])

    cp_small = [
        pltpu.make_async_copy(src, dst, sem_w.at[6 + i])
        for i, (src, dst) in enumerate([
            (shift_hbm, shift_ref), (ssmd_hbm, ssmd_ref), (b1_hbm, b1_ref),
            (b2_hbm, b2_ref), (c_hbm, c_ref)])
    ]

    for cp in cp_small:
        cp.start()
    cp_fwd.start()
    for cp in slab_copies(0):
        cp.start()
    cp_inv.start()
    for c in range(1, nslab):
        for cp in slab_copies(c):
            cp.start()
    cp_wm.start()
    cp_q.start()
    cp_w1.start()
    cp_w2.start()

    for cp in cp_small:
        cp.wait()
    sh_t = shift_ref[...].astype(f32)
    dvec = ssmd_ref[...].astype(f32).reshape(1, D)
    for c in range(nslab):
        sl = slice(c * _LANES, (c + 1) * _LANES)
        for j in range(4):
            taps[c, j] = jnp.broadcast_to(sh_t[j:j + 1, sl], (8, _LANES))
        taps[c, 4] = jnp.broadcast_to(dvec[:, sl], (8, _LANES))

    cp_fwd.wait()
    cp_inv.wait()

    def slab_body(c, carry):
        for cp in slab_copies(c):
            cp.wait()
        fmat = fwd[...]
        tap = [taps[c, j][0:1, :] for j in range(4)]
        prev = jnp.zeros((8, _LANES), f32)
        for j in range(nblk):
            rows = slice(j * _T, (j + 1) * _T)
            kc = kbuf[c, rows, :].astype(f32)
            ext = jnp.concatenate([prev, kc], axis=0)
            ks = kc * tap[0]
            for s in range(1, 4):
                ks = ks + ext[8 - s:8 - s + _T, :] * tap[s]
            prev = kc[_T - 8:, :]
            kv = ks * vbuf[c, rows, :].astype(f32)
            kvbuf[rows, :] = kv
            uspec[j] = jnp.dot(fmat, kv.astype(bf16), preferred_element_type=f32)
            kspec[j] = jax.lax.dot_general(
                fmat, sbuf[c, :, rows], (((1,), (1,)), ((), ())),
                preferred_element_type=f32)

        def make_pos_body(sign):
            def pos_body(p, carry2):
                re = pl.ds(pl.multiple_of(p * 8, 8), 8)
                im = pl.ds(pl.multiple_of(p * 8 + _T, 8), 8)
                kre = [kspec[m, re, :] for m in range(nblk)]
                kim = [kspec[m, im, :] for m in range(nblk)]
                cc, dd = [kre[0]], [kim[0]]
                for m in range(1, nblk):
                    if sign > 0:
                        cc.append(kre[m] - kim[m - 1])
                        dd.append(kim[m] + kre[m - 1])
                    else:
                        cc.append(kre[m] + kim[m - 1])
                        dd.append(kim[m] - kre[m - 1])
                a = [uspec[j, re, :] for j in range(nblk)]
                b = [uspec[j, im, :] for j in range(nblk)]
                p1 = _toeplitz([x + y for x, y in zip(a, b)], cc)
                p2 = _toeplitz(a, [y - x for x, y in zip(cc, dd)])
                for i in range(nblk):
                    yspec[i, im, :] = p1[i] + p2[i]
                p3 = _toeplitz(b, [x + y for x, y in zip(cc, dd)])
                for i in range(nblk):
                    yspec[i, re, :] = p1[i] - p3[i]
                return carry2
            return pos_body

        half = _T // 16
        jax.lax.fori_loop(0, half, make_pos_body(1), 0)
        jax.lax.fori_loop(half, 2 * half, make_pos_body(-1), 0)

        gmat = inv[...]
        dskip = taps[c, 4][0:1, :]
        for i in range(nblk):
            rows = slice(i * _T, (i + 1) * _T)
            y = jnp.dot(gmat, yspec[i].astype(bf16), preferred_element_type=f32)
            ybuf[c, rows, :] = y + kvbuf[rows, :] * dskip
        return carry

    jax.lax.fori_loop(0, nslab, slab_body, 0)

    cp_wm.wait()
    cv = c_ref[...].astype(f32)
    sc = cv * (1.0 / (1.0 + jnp.exp(-cv)))
    sc8 = jnp.broadcast_to(sc, (8, D)).astype(bf16)
    modbuf[...] = jnp.dot(sc8, wmbuf[...], preferred_element_type=f32)

    cp_q.wait()
    cp_w1.wait()
    cp_w2.wait()

    def out_copy(r):
        rows = pl.ds(pl.multiple_of(r * _ROWS, _ROWS), _ROWS)
        return pltpu.make_async_copy(obuf.at[rows, :], out_hbm.at[rows, :], sem_o.at[r])

    def row_body(r, carry):
        rows = pl.ds(pl.multiple_of(r * _ROWS, _ROWS), _ROWS)
        mod = [modbuf[0:1, j * D:(j + 1) * D] for j in range(6)]
        sa, ca, ga, sb, cb, gb = mod
        x = qbuf[rows, :].astype(f32)
        y = jnp.concatenate([ybuf[c, rows, :] for c in range(nslab)], axis=1)
        h = _layernorm(x) * (1.0 + ca) + sa
        x2 = x + ga * (h * y)
        h2 = _layernorm(x2) * (1.0 + cb) + sb
        a = jax.lax.dot_general(h2.astype(bf16), w1buf[...], (((1,), (1,)), ((), ())),
                                preferred_element_type=f32)
        a = _gelu(a + b1_ref[...].astype(f32).reshape(1, -1))
        o = jnp.dot(a.astype(bf16), w2buf[...], preferred_element_type=f32)
        o = x2 + gb * (o + b2_ref[...].astype(f32).reshape(1, D))
        obuf[rows, :] = o.astype(obuf.dtype)
        out_copy(r).start()
        return carry

    nrow = S // _ROWS
    jax.lax.fori_loop(0, nrow, row_body, 0)
    for r in range(nrow):
        out_copy(r).wait()


@jax.jit
def pallas_adaLN_cond__ssm_conv_h3__dense_activation_gelu__prompt_kernel(
    A_q: jax.Array,
    A_k: jax.Array,
    A_v: jax.Array,
    A_shift_k: jax.Array,
    A_ssm_k: jax.Array,
    A_ssm_D: jax.Array,
    B_x: jax.Array,
    B_w1: jax.Array,
    B_b1: jax.Array,
    B_w2: jax.Array,
    B_b2: jax.Array,
    c: jax.Array,
    w_mod: jax.Array,
):
    del B_x
    B, S, D = A_q.shape
    F = B_w1.shape[1]
    assert B == 1 and S % _ROWS == 0 and D % _LANES == 0
    nslab, nblk = D // _LANES, S // _T
    f32, bf16 = jnp.float32, jnp.bfloat16

    hbm = pl.BlockSpec(memory_space=pltpu.HBM)
    out = pl.pallas_call(
        _kernel,
        out_shape=jax.ShapeDtypeStruct((S, D), A_q.dtype),
        in_specs=[hbm] * 14,
        out_specs=hbm,
        scratch_shapes=[
            pltpu.VMEM((A_shift_k.shape[1], D), bf16),
            pltpu.VMEM((D,), bf16),
            pltpu.VMEM((F,), bf16),
            pltpu.VMEM((D,), bf16),
            pltpu.VMEM((1, D), bf16),
            pltpu.VMEM((nslab, S, _LANES), bf16),
            pltpu.VMEM((nslab, S, _LANES), bf16),
            pltpu.VMEM((nslab, _LANES, S), bf16),
            pltpu.VMEM((S, D), bf16),
            pltpu.VMEM((S, D), A_q.dtype),
            pltpu.VMEM((F, D), bf16),
            pltpu.VMEM((F, D), bf16),
            pltpu.VMEM((D, 6 * D), bf16),
            pltpu.VMEM((2 * _T, _T), bf16),
            pltpu.VMEM((_T, 2 * _T), bf16),
            pltpu.VMEM((nslab, 5, 8, _LANES), f32),
            pltpu.VMEM((S, _LANES), f32),
            pltpu.VMEM((nblk, 2 * _T, _LANES), f32),
            pltpu.VMEM((nblk, 2 * _T, _LANES), f32),
            pltpu.VMEM((nblk, 2 * _T, _LANES), f32),
            pltpu.VMEM((nslab, S, _LANES), f32),
            pltpu.VMEM((8, 6 * D), f32),
            pltpu.SemaphoreType.DMA((nslab,)),
            pltpu.SemaphoreType.DMA((nslab,)),
            pltpu.SemaphoreType.DMA((nslab,)),
            pltpu.SemaphoreType.DMA((11,)),
            pltpu.SemaphoreType.DMA((S // _ROWS,)),
        ],
        compiler_params=pltpu.CompilerParams(vmem_limit_bytes=100 * 1024 * 1024),
    )(
        A_q.reshape(S, D), A_k.reshape(S, D), A_v.reshape(S, D), A_shift_k.T, A_ssm_k,
        A_ssm_D, B_w1.T, B_b1, B_w2, B_b2, c, w_mod,
        jnp.asarray(_FWD_NP, dtype=bf16), jnp.asarray(_INV_NP, dtype=bf16),
    )
    return out.reshape(B, S, D)
```

```python
import functools

import jax
import jax.numpy as jnp
import numpy as np
import jax.experimental.pallas as pl
import jax.experimental.pallas.tpu as pltpu

_T = 128
_LANES = 128
_ROWS = 256
_EPS = 1e-5
_FCH = 256
_ICH = 128
_PIECE = 32


def _dft_matrices():
    k = np.concatenate([np.arange(0, _T, 2), np.arange(1, _T, 2)])
    t = np.arange(_T)
    phase = ((2 * k[:, None] + 1) * t[None, :]) % (4 * _T)
    ang = phase.astype(np.float64) * (2.0 * np.pi / (4 * _T))
    fwd = np.concatenate([np.cos(ang), -np.sin(ang)], axis=0)
    inv = fwd.T / _T
    return fwd.astype(np.float32), inv.astype(np.float32)


_FWD_NP, _INV_NP = _dft_matrices()


def _layernorm(x):
    m = jnp.mean(x, axis=-1, keepdims=True)
    d = x - m
    v = jnp.mean(d * d, axis=-1, keepdims=True)
    return d * jax.lax.rsqrt(v + _EPS)


def _gelu(x):
    c0 = float(np.sqrt(2.0 / np.pi))
    inner = x * (c0 + (c0 * 0.044715) * (x * x))
    hx = 0.5 * x
    return hx + hx * jnp.tanh(inner)


def _toeplitz_row(u, k, i):
    acc = u[0] * k[i]
    for j in range(1, i + 1):
        acc = acc + u[j] * k[i - j]
    return acc


def _interleave(*streams):
    streams = [[0.0, scale, gen] for gen, scale in streams]
    while streams:
        cur = min(streams, key=lambda e: e[0])
        cost = next(cur[2], None)
        if cost is None:
            streams.remove(cur)
        else:
            cur[0] += cost * cur[1]


def _kernel(q_hbm, k_hbm, v_hbm, shift_hbm, ssmk_hbm, ssmd_hbm, w1t_hbm, b1_hbm,
            w2_hbm, b2_hbm, c_hbm, wmod_hbm, fwd_hbm, inv_hbm, out_hbm,
            shift_ref, ssmd_ref, b1_ref, b2_ref, c_ref,
            kbuf, vbuf, sbuf, qbuf, obuf, w1buf, w2buf, wmbuf, fwd, inv,
            taps, uspec0, uspec1, kspec0, kspec1, yspec0, yspec1, ybuf, modbuf, hbuf, xbuf, b1f, b2f,
            sem_k, sem_v, sem_s, sem_w, sem_q, sem_o):
    S, D = qbuf.shape
    nslab = D // _LANES
    nblk = S // _T
    f32, bf16 = jnp.float32, jnp.bfloat16

    def slab_copies(c):
        lo = pl.multiple_of(c * _LANES, _LANES)
        return (
            pltpu.make_async_copy(k_hbm.at[:, pl.ds(lo, _LANES)], kbuf.at[c], sem_k.at[c]),
            pltpu.make_async_copy(v_hbm.at[:, pl.ds(lo, _LANES)], vbuf.at[c], sem_v.at[c]),
            pltpu.make_async_copy(ssmk_hbm.at[pl.ds(lo, _LANES), :], sbuf.at[c], sem_s.at[c]),
        )

    cp_fwd = pltpu.make_async_copy(fwd_hbm, fwd, sem_w.at[0])
    cp_inv = pltpu.make_async_copy(inv_hbm, inv, sem_w.at[1])
    cp_wm = pltpu.make_async_copy(wmod_hbm, wmbuf, sem_w.at[2])
    cp_w1 = pltpu.make_async_copy(w1t_hbm, w1buf, sem_w.at[3])
    cp_w2 = pltpu.make_async_copy(w2_hbm, w2buf, sem_w.at[4])
    nrow = S // _ROWS

    def q_copy(r):
        rows = pl.ds(pl.multiple_of(r * _ROWS, _ROWS), _ROWS)
        return pltpu.make_async_copy(q_hbm.at[rows, :], qbuf.at[rows, :], sem_q.at[r])

    cp_small = [
        pltpu.make_async_copy(src, dst, sem_w.at[6 + i])
        for i, (src, dst) in enumerate([
            (shift_hbm, shift_ref), (ssmd_hbm, ssmd_ref), (b1_hbm, b1_ref),
            (b2_hbm, b2_ref), (c_hbm, c_ref)])
    ]

    for cp in cp_small:
        cp.start()
    cp_fwd.start()
    for cp in slab_copies(0):
        cp.start()
    cp_inv.start()
    later = [[cp_wm], [q_copy(0), cp_w1], [cp_w2], [q_copy(r) for r in range(1, nrow)]]

    for cp in cp_small:
        cp.wait()
    sh_t = shift_ref[...].astype(f32)
    dvec = ssmd_ref[...].astype(f32).reshape(1, D)
    for c in range(nslab):
        sl = slice(c * _LANES, (c + 1) * _LANES)
        for j in range(4):
            taps[c, j] = jnp.broadcast_to(sh_t[j:j + 1, sl], (8, _LANES))
        taps[c, 4] = jnp.broadcast_to(dvec[:, sl], (8, _LANES))

    cp_fwd.wait()
    cp_inv.wait()

    uspec, kspec, yspec = (uspec0, uspec1), (kspec0, kspec1), (yspec0, yspec1)

    def forward(c, j):
        lo = j * _T
        rows = pl.ds(lo, _T)
        kc = kbuf[c, rows, :].astype(f32)
        if j > 0:
            prev = kbuf[c, pl.ds(lo - 16, 16), :].astype(f32)[8:, :]
        else:
            prev = jnp.zeros((8, _LANES), f32)
        ext = jnp.concatenate([prev, kc], axis=0)
        ks = kc * taps[c, 0][0:1, :]
        for t in range(1, 4):
            ks = ks + ext[8 - t:8 - t + _T, :] * taps[c, t][0:1, :]
        kv = ks * vbuf[c, rows, :].astype(f32)
        ybuf[c, rows, :] = kv * taps[c, 4][0:1, :]
        kv = kv.astype(bf16)
        yield 1
        for lo_r in range(0, 2 * _T, _FCH):
            part = slice(lo_r, lo_r + _FCH)
            kspec[c % 2][j, part, :] = jax.lax.dot_general(
                fwd[part, :], sbuf[c, :, rows], (((1,), (1,)), ((), ())),
                preferred_element_type=f32)
            yield 1
        for lo_r in range(0, 2 * _T, _FCH):
            part = slice(lo_r, lo_r + _FCH)
            uspec[c % 2][j, part, :] = jnp.dot(fwd[part, :], kv, preferred_element_type=f32)
            yield 1

    def inverse(c, i):
        spec = yspec[c % 2][i].astype(bf16)
        for lo_r in range(0, _T, _ICH):
            part = pl.ds(i * _T + lo_r, _ICH)
            y = jnp.dot(inv[lo_r:lo_r + _ICH, :], spec, preferred_element_type=f32)
            ybuf[c, part, :] = ybuf[c, part, :] + y
            yield 1

    def accumulate(c, p, sign):
        us, ks_, ys = uspec[c % 2], kspec[c % 2], yspec[c % 2]
        re = pl.ds(pl.multiple_of(p * 8, 8), 8)
        im = pl.ds(pl.multiple_of(p * 8 + _T, 8), 8)
        kre = [ks_[m, re, :] for m in range(nblk)]
        kim = [ks_[m, im, :] for m in range(nblk)]
        cc, dd = [kre[0]], [kim[0]]
        for m in range(1, nblk):
            if sign > 0:
                cc.append(kre[m] - kim[m - 1])
                dd.append(kim[m] + kre[m - 1])
            else:
                cc.append(kre[m] + kim[m - 1])
                dd.append(kim[m] - kre[m - 1])
        a = [us[j, re, :] for j in range(nblk)]
        b = [us[j, im, :] for j in range(nblk)]
        ab = [x + y for x, y in zip(a, b)]
        p1 = []
        for i in range(nblk):
            p1.append(_toeplitz_row(ab, cc, i))
            yield i + 1
        dc = [y - x for x, y in zip(cc, dd)]
        for i in range(nblk):
            ys[i, im, :] = p1[i] + _toeplitz_row(a, dc, i)
            yield i + 1
        cd = [x + y for x, y in zip(cc, dd)]
        for i in range(nblk):
            ys[i, re, :] = p1[i] - _toeplitz_row(b, cd, i)
            yield i + 1

    def run(lo, hi, fn):
        def body(i, carry):
            _interleave(*fn(i))
            return carry
        jax.lax.fori_loop(lo, hi, body, 0)

    def drain(gens):
        for g in gens:
            for _ in g:
                pass

    for c in range(nslab):
        for cp in slab_copies(c):
            cp.wait()
        starts = list(slab_copies(c + 1)) if c + 1 < nslab else []
        if c > 0 or nslab == 1:
            starts += later.pop(0)
        if c + 1 == nslab:
            starts += sum(later, [])
        for cp in starts:
            cp.start()
        drain(forward(c, j) for j in range(nblk))
        run(0, nblk // 2, lambda p: [(accumulate(c, p, 1), 1)])
        run(nblk // 2, nblk, lambda p: [(accumulate(c, p, -1), 1)])
        drain(inverse(c, i) for i in range(nblk))

    cp_wm.wait()
    cv = c_ref[...].astype(f32)
    sc = cv * (1.0 / (1.0 + jnp.exp(-cv)))
    sc8 = jnp.broadcast_to(sc, (8, D)).astype(bf16)
    modbuf[...] = jnp.dot(sc8, wmbuf[...], preferred_element_type=f32)

    cp_w1.wait()
    cp_w2.wait()

    def out_copy(r):
        rows = pl.ds(pl.multiple_of(r * _ROWS, _ROWS), _ROWS)
        return pltpu.make_async_copy(obuf.at[rows, :], out_hbm.at[rows, :], sem_o.at[r])

    def mod(j):
        return modbuf[0:1, j * D:(j + 1) * D]

    def prepare(r, piece, after=None):
        rows = pl.ds(pl.multiple_of(r * _ROWS + piece * _PIECE, _PIECE), _PIECE)
        x = qbuf[rows, :].astype(f32)
        if after is not None:
            x = jnp.maximum(x, jnp.minimum(after, -jnp.inf))
        y = jnp.concatenate([ybuf[c, rows, :] for c in range(nslab)], axis=1)
        h = _layernorm(x) * (1.0 + mod(1)) + mod(0)
        x2 = x + mod(2) * (h * y)
        h2 = _layernorm(x2) * (1.0 + mod(4)) + mod(3)
        hbuf[rows, :] = h2.astype(bf16)
        xbuf[rows, :] = x2

    npiece = _ROWS // _PIECE
    F = w2buf.shape[0]

    def row_body(r, carry):
        nxt = jnp.minimum(r + 1, nrow - 1)

        @pl.when(r + 1 < nrow)
        def _():
            q_copy(nxt).wait()

        rows = pl.ds(pl.multiple_of(r * _ROWS, _ROWS), _ROWS)
        h2 = hbuf[rows, :]
        acts, after = [], None
        for n, lo in enumerate(range(0, F, 256)):
            cols = slice(lo, min(lo + 256, F))
            a = jax.lax.dot_general(h2, w1buf[cols, :], (((1,), (1,)), ((), ())),
                                    preferred_element_type=f32)
            acts.append(_gelu(a + b1f[0:1, cols]).astype(bf16))
            for piece in range(npiece):
                if piece * 7 // npiece == n:
                    prepare(nxt, piece, a[0:1, 0:1])
        o = jnp.dot(jnp.concatenate(acts, axis=1), w2buf[...], preferred_element_type=f32)
        o = xbuf[rows, :] + mod(5) * (o + b2f[...])
        obuf[rows, :] = o.astype(obuf.dtype)
        out_copy(r).start()
        return carry

    b1f[...] = b1_ref[...].astype(f32).reshape(1, F)
    b2f[...] = b2_ref[...].astype(f32).reshape(1, D)
    q_copy(0).wait()
    for piece in range(npiece):
        prepare(0, piece)
    jax.lax.fori_loop(0, nrow, row_body, 0)
    for r in range(nrow):
        out_copy(r).wait()


@jax.jit
def pallas_adaLN_cond__ssm_conv_h3__dense_activation_gelu__prompt_kernel(
    A_q: jax.Array,
    A_k: jax.Array,
    A_v: jax.Array,
    A_shift_k: jax.Array,
    A_ssm_k: jax.Array,
    A_ssm_D: jax.Array,
    B_x: jax.Array,
    B_w1: jax.Array,
    B_b1: jax.Array,
    B_w2: jax.Array,
    B_b2: jax.Array,
    c: jax.Array,
    w_mod: jax.Array,
):
    del B_x
    B, S, D = A_q.shape
    F = B_w1.shape[1]
    assert B == 1 and S % _ROWS == 0 and D % _LANES == 0
    nslab, nblk = D // _LANES, S // _T
    f32, bf16 = jnp.float32, jnp.bfloat16

    hbm = pl.BlockSpec(memory_space=pltpu.HBM)
    out = pl.pallas_call(
        _kernel,
        out_shape=jax.ShapeDtypeStruct((S, D), A_q.dtype),
        in_specs=[hbm] * 14,
        out_specs=hbm,
        scratch_shapes=[
            pltpu.VMEM((A_shift_k.shape[1], D), bf16),
            pltpu.VMEM((D,), bf16),
            pltpu.VMEM((F,), bf16),
            pltpu.VMEM((D,), bf16),
            pltpu.VMEM((1, D), bf16),
            pltpu.VMEM((nslab, S, _LANES), bf16),
            pltpu.VMEM((nslab, S, _LANES), bf16),
            pltpu.VMEM((nslab, _LANES, S), bf16),
            pltpu.VMEM((S, D), bf16),
            pltpu.VMEM((S, D), A_q.dtype),
            pltpu.VMEM((F, D), bf16),
            pltpu.VMEM((F, D), bf16),
            pltpu.VMEM((D, 6 * D), bf16),
            pltpu.VMEM((2 * _T, _T), bf16),
            pltpu.VMEM((_T, 2 * _T), bf16),
            pltpu.VMEM((nslab, 5, 8, _LANES), f32),
            *[pltpu.VMEM((nblk, 2 * _T, _LANES), f32)] * 6,
            pltpu.VMEM((nslab, S, _LANES), f32),
            pltpu.VMEM((8, 6 * D), f32),
            pltpu.VMEM((S, D), bf16),
            pltpu.VMEM((S, D), f32),
            pltpu.VMEM((1, F), f32),
            pltpu.VMEM((1, D), f32),
            pltpu.SemaphoreType.DMA((nslab,)),
            pltpu.SemaphoreType.DMA((nslab,)),
            pltpu.SemaphoreType.DMA((nslab,)),
            pltpu.SemaphoreType.DMA((11,)),
            pltpu.SemaphoreType.DMA((S // _ROWS,)),
            pltpu.SemaphoreType.DMA((S // _ROWS,)),
        ],
        compiler_params=pltpu.CompilerParams(vmem_limit_bytes=100 * 1024 * 1024),
    )(
        A_q.reshape(S, D), A_k.reshape(S, D), A_v.reshape(S, D), A_shift_k.T, A_ssm_k,
        A_ssm_D, B_w1.T, B_b1, B_w2, B_b2, c, w_mod,
        jnp.asarray(_FWD_NP, dtype=bf16), jnp.asarray(_INV_NP, dtype=bf16),
    )
    return out.reshape(B, S, D)
```
